```python
import os as _os
_os.environ.setdefault("JAX_PLATFORMS", "cpu")
import jax
import jax.numpy as jnp

def _softmax(x, axis=-1):
    return jax.nn.softmax(x, axis=axis)
def _gelu(x):
    return jax.nn.gelu(x, approximate=True)
def _silu(x):
    return jax.nn.silu(x)
def _sigmoid(x):
    return jax.nn.sigmoid(x)
def _layernorm(x, axis=-1, eps=1e-5):
    m = jnp.mean(x, axis=axis, keepdims=True)
    v = jnp.var(x, axis=axis, keepdims=True)
    return (x - m) / jnp.sqrt(v + eps)
def _scatter_add(tgt, idx, src, axis=0):
    return tgt.at[idx].add(src)
def _segment_sum(src, seg, n):
    return jax.ops.segment_sum(src, seg, n)
class _Rng:
    def __init__(self, key):
        self._k = key
    def _next(self):
        self._k, sub = jax.random.split(self._k)
        return sub
    def normal(self, shape):
        return jax.random.normal(self._next(), shape, dtype=jnp.bfloat16)
    def randint(self, lo, hi, shape):
        return jax.random.randint(self._next(), shape, lo, hi, dtype=jnp.int32)
    def uniform(self, shape, lo=0.0, hi=1.0):
        return jax.random.uniform(self._next(), shape, jnp.bfloat16, lo, hi)
    def permutation(self, n):
        return jax.random.permutation(self._next(), n)


kernel_name = 'standalone__gqa_block_cached__near_ridge'

def setup_inputs():
    _rng = _Rng(jax.random.key(int.from_bytes(__import__("os").urandom(4), "little")))
    _w = (lambda a: (lambda t: t.astype(jnp.bfloat16) if jnp.issubdtype(t.dtype, jnp.floating) else t)(jnp.asarray(a)))
    B, Sq, D = 8, 96, 640
    Hq, Hkv, Sk, Dh = 32, 32, 512, 128
    assert Hq % Hkv == 0, (Hq, Hkv)
    return {
        "x": _w((lambda *s: _rng.normal(s) * 0.2)(B, Sq, D)),
        "k_cache": _w((lambda *s: _rng.normal(s) * 3.2)(B, Hkv, Sk, Dh)),
        "v_cache": _w((lambda *s: _rng.normal(s) * 0.05)(B, Hkv, Sk, Dh)),
        "wq": _w((lambda *s: _rng.normal(s) * 0.2)(D, Hq * Dh) * (D ** -0.5)),
        "wo": _w((lambda *s: _rng.normal(s) * 0.05)(Hq * Dh, D) * ((Hq * Dh) ** -0.5)),
    }

def reference(x, k_cache, v_cache, wq, wo):
    B, Sq, D = x.shape
    Hq, Dh = 32, 128
    Hkv = k_cache.shape[1]
    rep = Hq // Hkv
    q = (lambda x, *d: x.transpose(*d))((x @ wq).reshape(B, Sq, Hq, Dh), 0, 2, 1, 3)
    k = jnp.repeat(k_cache, rep, axis=1)
    v = jnp.repeat(v_cache, rep, axis=1)
    scores = jnp.einsum("bhqd,bhkd->bhqk", q, k) * (Dh ** -0.5)
    p = _softmax(scores, axis=-1)
    o = jnp.einsum("bhqk,bhkd->bhqd", p, v)
    return (lambda x, *d: x.transpose(*d))(o, 0, 2, 1, 3).reshape(B, Sq, Hq * Dh) @ wo
```

```python
import functools, math
import jax, jax.numpy as jnp
from jax import lax
from jax.experimental import pallas as pl
from jax.experimental.pallas import tpu as pltpu

B,Sq,D,H,Sk,Dh = 8,96,640,32,512,128
LOG2E = math.log2(math.e)
f32, bf16 = jnp.float32, jnp.bfloat16

def make(G=4, order='skew', flags=None, dma=True):
    NG = H//G
    scale = (Dh ** -0.5) * LOG2E
    def kernel(x_hbm, k_hbm, v_hbm, wq_hbm, wo_hbm, out_hbm,
               x_v, wq_v, wo_v, k_v, v_v, o_v, acc_v, out_v, sems):
        def cp_x(): return pltpu.make_async_copy(x_hbm, x_v, sems.at[0])
        def cp_wq(g): return pltpu.make_async_copy(wq_hbm.at[:, pl.ds(g*G*Dh, G*Dh)], wq_v.at[g], sems.at[1+4*g])
        def cp_k(g): return pltpu.make_async_copy(k_hbm.at[:, pl.ds(g*G, G)], k_v.at[g], sems.at[2+4*g])
        def cp_v(g): return pltpu.make_async_copy(v_hbm.at[:, pl.ds(g*G, G)], v_v.at[g], sems.at[3+4*g])
        def cp_wo(g): return pltpu.make_async_copy(wo_hbm.at[pl.ds(g*G*Dh, G*Dh), :], wo_v.at[g], sems.at[4+4*g])
        if dma:
            cp_x().start()
            for g in range(NG):
                cp_wq(g).start(); cp_k(g).start(); cp_v(g).start(); cp_wo(g).start()
        acc_v[...] = jnp.zeros_like(acc_v)
        if dma: cp_x().wait()

        def qproj(g, b):
            q = jnp.dot(x_v[b], wq_v[g], preferred_element_type=f32) * scale
            return q.astype(bf16)
        def qk(g, b, j, q):
            return lax.dot_general(q[:, j*Dh:(j+1)*Dh], k_v[g, b, j], (((1,),(1,)),((),())), preferred_element_type=f32)
        def sm_pv(g, b, j, s):
            m = jnp.max(s, axis=-1, keepdims=True)
            p = jnp.exp2(s - m)
            l = jnp.sum(p, axis=-1, keepdims=True)
            o = jnp.dot(p.astype(bf16), v_v[g, b, j], preferred_element_type=f32)
            o = o * (1.0 / l)
            o_v[b, :, j*Dh:(j+1)*Dh] = o.astype(bf16)
        def oproj(g, b):
            y = jnp.dot(o_v[b], wo_v[g], preferred_element_type=f32)
            acc_v[b] += y

        def body(g, _):
            if dma:
                cp_wq(g).wait(); cp_k(g).wait(); cp_v(g).wait(); cp_wo(g).wait()
            N = B*G
            if order == 'plain':
                for b in range(B):
                    q = qproj(g, b)
                    for j in range(G):
                        sm_pv(g, b, j, qk(g, b, j, q))
                    oproj(g, b)
            elif order == 'swp':
                qs = {}
                qs[0] = qproj(g, 0)
                s = qk(g, 0, 0, qs[0])
                for n in range(N):
                    b, j = divmod(n, G)
                    if n+1 < N:
                        b1, j1 = divmod(n+1, G)
                        if j1 == 0: qs[b1] = qproj(g, b1)
                        s_next = qk(g, b1, j1, qs[b1])
                    sm_pv(g, b, j, s)
                    if j == G-1: oproj(g, b)
                    s = s_next
            elif order == 'skew':
                qs = {}
                qs[0] = qproj(g, 0)
                s = qk(g, 0, 0, qs[0])
                for n in range(N):
                    b, j = divmod(n, G)
                    if n+1 < N:
                        b1, j1 = divmod(n+1, G)
                        s_next = qk(g, b1, j1, qs[b1])
                    if j == 0 and b+1 < B: qs[b+1] = qproj(g, b+1)
                    if j == 2 and b >= 1: oproj(g, b-1)
                    sm_pv(g, b, j, s)
                    s = s_next
                oproj(g, B-1)
            return None
        lax.fori_loop(0, NG, body, None)
        out_v[...] = acc_v[...].astype(bf16)
        oc = pltpu.make_async_copy(out_v, out_hbm, sems.at[1+4*NG])
        oc.start(); oc.wait()

    def fn(x, k, v, wq, wo):
        return pl.pallas_call(kernel,
            in_specs=[pl.BlockSpec(memory_space=pl.ANY)]*5,
            out_specs=pl.BlockSpec(memory_space=pl.ANY),
            out_shape=jax.ShapeDtypeStruct((B,Sq,D), bf16),
            scratch_shapes=[pltpu.VMEM((B,Sq,D), bf16),
                pltpu.VMEM((NG,D,G*Dh), bf16), pltpu.VMEM((NG,G*Dh,D), bf16),
                pltpu.VMEM((NG,B,G,Sk,Dh), bf16), pltpu.VMEM((NG,B,G,Sk,Dh), bf16),
                pltpu.VMEM((B,Sq,G*Dh), bf16), pltpu.VMEM((B,Sq,D), f32), pltpu.VMEM((B,Sq,D), bf16),
                pltpu.SemaphoreType.DMA((4*NG+2,))],
            compiler_params=pltpu.CompilerParams(vmem_limit_bytes=120*1024*1024, flags=flags),
        )(x,k,v,wq,wo)
    return fn


_kernel_impl = make(4, 'skew')


@jax.jit
def pallas_standalone__gqa_block_cached__near_ridge_kernel(x, k_cache, v_cache, wq, wo):
    return _kernel_impl(x, k_cache, v_cache, wq, wo)
```

```python
import math

import jax
import jax.numpy as jnp
from jax import lax
import jax.experimental.pallas as pl
import jax.experimental.pallas.tpu as pltpu

G = 4

N_LOOP = 5
PIECES = {
    5: ((0, 4), (4, 4)),
    6: ((0, 2), (2, 2), (4, 2), (6, 1), (7, 1)),
    7: ((0, 1), (1, 1), (2, 1), (3, 1)),
}
N_SPLIT = 4
O_SLOT = 2


@jax.jit
def pallas_standalone__gqa_block_cached__near_ridge_kernel(
    x: jax.Array,
    k_cache: jax.Array,
    v_cache: jax.Array,
    wq: jax.Array,
    wo: jax.Array,
):
    B, Sq, D = x.shape
    _, H, Sk, Dh = k_cache.shape
    assert wq.shape == (D, H * Dh) and wo.shape == (H * Dh, D) and H % G == 0
    NG = H // G
    GD = G * Dh
    M = B * Sq
    LAST = NG - 1
    B_SPLIT = B - N_SPLIT
    C_LATE = D - 128
    assert sorted(PIECES) == list(range(N_LOOP, NG))
    for g, pieces in PIECES.items():
        end = 0
        for b0, nb in pieces:
            assert b0 == end
            end += nb
        assert end == (B_SPLIT if g == LAST else B)

    f32 = jnp.float32
    dt = x.dtype
    q_scale = (Dh**-0.5) * math.log2(math.e)

    sem_index = {}
    for key in ("x", "wq", "wo"):
        sem_index[key] = len(sem_index)
    loop_sem = len(sem_index)
    for g in range(N_LOOP):
        for w in range(2):
            sem_index["loop", g, w] = len(sem_index)
    for g in range(N_LOOP, NG):
        for b0, _ in PIECES[g]:
            for w in range(2):
                sem_index["piece", g, b0, w] = len(sem_index)
    for b in range(B_SPLIT, B):
        for w in range(2):
            sem_index["split", b, w] = len(sem_index)
    for key in ("out_first", "out_mid", "out_last"):
        sem_index[key] = len(sem_index)

    def kernel(x_hbm, k_hbm, v_hbm, wq_hbm, wo_hbm, out_hbm,
               x_v, wq_v, wo_v, k_v, v_v, q_v, o_v, p_v, acc_v, out_v, sems):
        def copy(src, dst, sem):
            return pltpu.make_async_copy(src, dst, sems.at[sem])

        def kv_copy(w, g, b0, nb, sem):
            src, dst = ((k_hbm, k_v), (v_hbm, v_v))[w]
            sl = (pl.ds(b0, nb), pl.ds(g * G, G))
            return copy(src.at[sl], dst.at[sl], sem)

        def loop_copies(g):
            return [kv_copy(w, g, 0, B, loop_sem + 2 * g + w) for w in range(2)]

        def piece_copies(g, b0):
            nb = dict(PIECES[g])[b0]
            return [kv_copy(w, g, b0, nb, sem_index["piece", g, b0, w]) for w in range(2)]

        def split_copy(w, b):
            return kv_copy(w, LAST, b, 1, sem_index["split", b, w])

        def out_copy(key):
            b0, nb = {"out_first": (0, 1), "out_mid": (1, B - 2), "out_last": (B - 1, 1)}[key]
            return copy(out_v.at[pl.ds(b0, nb)], out_hbm.at[pl.ds(b0, nb)], sem_index[key])

        x_copy = copy(x_hbm, x_v, sem_index["x"])
        wq_copy = copy(wq_hbm, wq_v, sem_index["wq"])
        wo_copy = copy(wo_hbm, wo_v, sem_index["wo"])

        x_copy.start()
        wq_copy.start()
        for g in range(N_LOOP):
            for c in loop_copies(g):
                c.start()
            if g == 0:
                wo_copy.start()
        for g in range(N_LOOP, NG):
            for b0, _ in PIECES[g]:
                for c in piece_copies(g, b0):
                    c.start()
        for b in range(B_SPLIT, B):
            split_copy(0, b).start()
            split_copy(1, b).start()

        acc_v[...] = jnp.zeros_like(acc_v)

        x_copy.wait()
        wq_copy.wait()

        def group_cols(g):
            start = g * GD
            if not isinstance(g, int):
                start = pl.multiple_of(start, GD)
            return pl.ds(start, GD)

        def q_projection(g, carry):
            q = jnp.dot(x_v[...], wq_v[:, group_cols(g)], preferred_element_type=f32)
            q = (q * q_scale).astype(dt)
            for j in range(G):
                q_v[g, j] = q[:, j * Dh:(j + 1) * Dh]
            return carry

        lax.fori_loop(0, NG, q_projection, None)

        def scores(g, b, j):
            return lax.dot_general(
                q_v[g, j, b * Sq:(b + 1) * Sq, :], k_v[b, g * G + j],
                (((1,), (1,)), ((), ())), preferred_element_type=f32)

        def softmax(s):
            m = jnp.max(s, axis=-1, keepdims=True)
            p = jnp.exp2(s - m)
            l = jnp.sum(p, axis=-1, keepdims=True)
            return p.astype(dt), l

        def attend(g, b, j, p, l):
            o = jnp.dot(p, v_v[b, g * G + j], preferred_element_type=f32)
            o_v[b, :, j * Dh:(j + 1) * Dh] = (o * (1.0 / l)).astype(dt)

        def out_projection(g, b, c0=0, c1=D):
            y = jnp.dot(o_v[b], wo_v[group_cols(g), c0:c1], preferred_element_type=f32)
            if isinstance(g, int) and g == LAST:
                out_v[b, :, c0:c1] = (acc_v[b, :, c0:c1] + y).astype(dt)
            else:
                acc_v[b, :, c0:c1] += y

        wo_copy.wait()

        def group_body(g, carry):
            for c in loop_copies(g):
                c.wait()
            s = scores(g, 0, 0)
            for n in range(B * G):
                b, j = divmod(n, G)
                if n + 1 < B * G:
                    s_next = scores(g, *divmod(n + 1, G))
                if j == O_SLOT and b >= 1:
                    out_projection(g, b - 1)
                attend(g, b, j, *softmax(s))
                s = s_next
            out_projection(g, B - 1)
            return carry

        lax.fori_loop(0, N_LOOP, group_body, None)

        slots = [(g, b, j) for g in range(N_LOOP, NG) for b in range(B) for j in range(G)]
        slots = slots[:-G * N_SPLIT]
        last_piece = slots[-1][:2]
        finished = []

        def flush():
            while finished:
                out_projection(*finished.pop(0))

        for c in piece_copies(N_LOOP, 0):
            c.wait()
        s = scores(*slots[0])
        for i, (g, b, j) in enumerate(slots):
            if i + 1 < len(slots):
                g1, b1, j1 = slots[i + 1]
                if j1 == 0 and b1 in dict(PIECES[g1]):
                    if (g1, b1) == last_piece:
                        attend(g, b, j, *softmax(s))
                        finished.append((g, b))
                        flush()
                        for c in piece_copies(g1, b1):
                            c.wait()
                        s = scores(g1, b1, j1)
                        continue
                    for c in piece_copies(g1, b1):
                        c.wait()
                s_next = scores(g1, b1, j1)
            if j == O_SLOT:
                flush()
            attend(g, b, j, *softmax(s))
            if j == G - 1:
                finished.append((g, b))
            s = s_next

        for b in range(B_SPLIT, B):
            final = b == B - 1
            if final:
                (gp, bp), = finished
                out_projection(gp, bp, 0, C_LATE)
            else:
                flush()
            split_copy(0, b).wait()
            if final:
                out_copy("out_first").start()
            s = scores(LAST, b, 0)
            sums = []
            for j in range(G):
                if j + 1 < G:
                    s_next = scores(LAST, b, j + 1)
                if final and j == 1:
                    out_projection(gp, bp, C_LATE, D)
                    finished.clear()
                    out_copy("out_mid").start()
                p, l = softmax(s)
                p_v[j] = p
                sums.append(l)
                s = s_next
            split_copy(1, b).wait()
            for j in range(G):
                attend(LAST, b, j, p_v[j], sums[j])
            finished.append((LAST, b))
        flush()
        out_copy("out_last").start()
        for key in ("out_first", "out_mid", "out_last"):
            out_copy(key).wait()

    return pl.pallas_call(
        kernel,
        in_specs=[pl.BlockSpec(memory_space=pl.ANY)] * 5,
        out_specs=pl.BlockSpec(memory_space=pl.ANY),
        out_shape=jax.ShapeDtypeStruct((B, Sq, D), dt),
        scratch_shapes=[
            pltpu.VMEM((M, D), dt),
            pltpu.VMEM((D, H * Dh), dt),
            pltpu.VMEM((H * Dh, D), dt),
            pltpu.VMEM((B, H, Sk, Dh), dt),
            pltpu.VMEM((B, H, Sk, Dh), dt),
            pltpu.VMEM((NG, G, M, Dh), dt),
            pltpu.VMEM((B, Sq, GD), dt),
            pltpu.VMEM((G, Sq, Sk), dt),
            pltpu.VMEM((B, Sq, D), f32),
            pltpu.VMEM((B, Sq, D), dt),
            pltpu.SemaphoreType.DMA((len(sem_index),)),
        ],
        compiler_params=pltpu.CompilerParams(
            vmem_limit_bytes=120 * 1024 * 1024,
            disable_semaphore_checks=True,
        ),
    )(x.reshape(M, D), k_cache, v_cache, wq, wo)
```
